```python
import jax
import jax.numpy as jnp

def _softmax(x, axis=-1):
    return jax.nn.softmax(x, axis=axis)
def _gelu(x):
    return jax.nn.gelu(x, approximate=True)
def _silu(x):
    return jax.nn.silu(x)
def _sigmoid(x):
    return jax.nn.sigmoid(x)
def _layernorm(x, axis=-1, eps=1e-5):
    m = jnp.mean(x, axis=axis, keepdims=True)
    v = jnp.var(x, axis=axis, keepdims=True)
    return (x - m) / jnp.sqrt(v + eps)
def _scatter_add(tgt, idx, src, axis=0):
    return tgt.at[idx].add(src)
def _segment_sum(src, seg, n):
    return jax.ops.segment_sum(src, seg, n)
class _Rng:
    def __init__(self, key):
        self._k = key
    def _next(self):
        self._k, sub = jax.random.split(self._k)
        return sub
    def normal(self, shape):
        return jax.random.normal(self._next(), shape, dtype=jnp.bfloat16)
    def randint(self, lo, hi, shape):
        return jax.random.randint(self._next(), shape, lo, hi, dtype=jnp.int32)
    def uniform(self, shape, lo=0.0, hi=1.0):
        return jax.random.uniform(self._next(), shape, jnp.bfloat16, lo, hi)
    def permutation(self, n):
        return jax.random.permutation(self._next(), n)


kernel_name = 'recurrent_scan__compressed_kv_cla__dense_activation_gelu__decode'

def setup_inputs():
    _rng = _Rng(jax.random.key(int.from_bytes(__import__("os").urandom(4), "little")))
    _w = (lambda a: (lambda t: t.astype(jnp.bfloat16) if jnp.issubdtype(t.dtype, jnp.floating) else t)(jnp.asarray(a)))
    def _A_setup():
        B, H, Sq, Sk, D, M = 2, 32, 1, 16384, 128, 512
        Dc = 4 * D
        return {
            "x": _w((lambda *s: _rng.normal(s) * 0.05)(B, Sq, M)),
            "c_kv": _w((lambda *s: _rng.normal(s) * 0.05)(B, Sk, Dc)),
            "w_q": _w((lambda *s: _rng.normal(s) * 0.05)(M, H, D) * (M ** -0.5)),
            "w_uk": _w((lambda *s: _rng.normal(s) * 0.05)(Dc, H, D) * (Dc ** -0.5)),
            "w_uv": _w((lambda *s: _rng.normal(s) * 0.05)(Dc, H, D) * (Dc ** -0.5)),
            "w_o": _w((lambda *s: _rng.normal(s) * 0.05)(H, D, M) * ((H * D) ** -0.5)),
        }
    _A_in = _A_setup()

    def _B_setup():
        B, S, D, F = 2, 1, 512, 1792
        return {
            "x": _w((lambda *s: _rng.normal(s) * 0.05)(B, S, D)),
            "w1": _w((lambda *s: _rng.normal(s) * 0.05)(D, F) * (D ** -0.5)),
            "b1": _w((lambda *s: _rng.normal(s) * 0.05)(F) * 0.01),
            "w2": _w((lambda *s: _rng.normal(s) * 0.05)(F, D) * (F ** -0.5)),
            "b2": _w((lambda *s: _rng.normal(s) * 0.05)(D) * 0.01),
        }
    _B_in = _B_setup()

    return {
        "A_x": _A_in["x"],
        "A_c_kv": _A_in["c_kv"],
        "A_w_q": _A_in["w_q"],
        "A_w_uk": _A_in["w_uk"],
        "A_w_uv": _A_in["w_uv"],
        "A_w_o": _A_in["w_o"],
        "B_x": _B_in["x"],
        "B_w1": _B_in["w1"],
        "B_b1": _B_in["b1"],
        "B_w2": _B_in["w2"],
        "B_b2": _B_in["b2"],
    }

def reference(A_x, A_c_kv, A_w_q, A_w_uk, A_w_uv, A_w_o, B_x, B_w1, B_b1, B_w2, B_b2):
    def _A_ref(x, c_kv, w_q, w_uk, w_uv, w_o):
        B, Sq, M = x.shape[0], x.shape[1], x.shape[2]
        Sk = c_kv.shape[1]
        H, D = w_q.shape[1], w_q.shape[2]
        q = jnp.einsum("bqm,mhd->bhqd", x, w_q)
        k = jnp.einsum("bkc,chd->bhkd", c_kv, w_uk)
        v = jnp.einsum("bkc,chd->bhkd", c_kv, w_uv)
        scores = jnp.einsum("bhqd,bhkd->bhqk", q, k) * (D ** -0.5)
        off = Sk - Sq
        qi = jnp.arange(Sq)[:, None]
        kj = jnp.arange(Sk)[None, :]
        cmask = kj <= (qi + off)
        scores = jnp.where(cmask[None, None], scores, -1e9)
        p = _softmax(scores, axis=-1)
        ctx = jnp.einsum("bhqk,bhkd->bhqd", p, v)
        return jnp.einsum("bhqd,hdm->bqm", ctx, w_o)

    def _B_ref(x, w1, b1, w2, b2):
        h = jnp.einsum("bsd,df->bsf", x, w1) + b1
        h = _gelu(h)
        return jnp.einsum("bsf,fd->bsd", h, w2) + b2

    x = A_x
    xn = _layernorm(x, axis=-1)
    s = _A_ref(xn, A_c_kv, A_w_q, A_w_uk, A_w_uv, A_w_o)
    g = _silu(_B_ref(xn, B_w1, B_b1, B_w2, B_b2))
    return x + s * g
```

```python
import jax
import jax.numpy as jnp
from jax import lax
import jax.experimental.pallas as pl
import jax.experimental.pallas.tpu as pltpu

LOG2E = 1.4426950408889634
BF16 = jnp.bfloat16
F32 = jnp.float32
U32 = jnp.uint32
NT = (((1,), (1,)), ((), ()))

TK = 1024
LANES = 128


def _kv_splits(sk):
    return (sk,), (sk // 2, sk // 4, sk // 4)


def _wo_splits(h):
    return (0, h * 5 // 8, h * 7 // 8, h - 1, h)


@jax.jit
def pallas_recurrent_scan__compressed_kv_cla__dense_activation_gelu__decode_kernel(
    A_x: jax.Array,
    A_c_kv: jax.Array,
    A_w_q: jax.Array,
    A_w_uk: jax.Array,
    A_w_uv: jax.Array,
    A_w_o: jax.Array,
    B_x: jax.Array,
    B_w1: jax.Array,
    B_b1: jax.Array,
    B_w2: jax.Array,
    B_b2: jax.Array,
):
    del B_x
    B, SQ, M = A_x.shape
    _, SK, DC = A_c_kv.shape
    _, H, D = A_w_q.shape
    F = B_w1.shape[1]
    assert B == 2 and SQ == 1 and D == LANES and H % 8 == 0 and M == DC
    assert DC % LANES == 0 and SK % (4 * TK) == 0
    CT = DC // LANES
    KV_SPLITS = _kv_splits(SK)
    WO_SPLITS = _wo_splits(H)
    NWO = len(WO_SPLITS) - 1
    SEM_KV = (2, 2 + len(KV_SPLITS[0]))
    SEM_WO = SEM_KV[1] + len(KV_SPLITS[1])
    NSEM = SEM_WO + NWO

    def head_pair(w_ref, grp, pj):
        u_ref = w_ref.bitcast(U32)
        n = u_ref.shape[0]
        sub = u_ref.at[pl.ds(pl.multiple_of(4 * grp, 4), n - (H // 2 - 4)), :]
        u = sub[pl.ds(pj, DC, stride=H // 2), :]
        lo = pltpu.bitcast(u << 16, F32).astype(BF16)
        hi = pltpu.bitcast(u & jnp.uint32(0xFFFF0000), F32).astype(BF16)
        return lo, hi

    def kernel(x_hbm, kv_hbm, wq_hbm, wuk_hbm, wuv_hbm, wo_hbm,
               w1_hbm, b1_hbm, w2_hbm, b2_hbm,
               o_ref,
               x_v, kv_v, wq_v, wuk_v, wuv_v, wo_v, w1_v, b1_v, w2_v, b2_v,
               qa_v, qb_v, olat_v, ctx_v, sems):
        cp = pltpu.make_async_copy

        def kv_copy(b, j):
            r = pl.ds(sum(KV_SPLITS[b][:j]), KV_SPLITS[b][j])
            return cp(kv_hbm.at[b, r], kv_v.at[b, r], sems.at[SEM_KV[b] + j])

        def wo_copy(i):
            r = pl.ds(WO_SPLITS[i], WO_SPLITS[i + 1] - WO_SPLITS[i])
            return cp(wo_hbm.at[r], wo_v.at[r], sems.at[SEM_WO + i])

        q_copies = [
            cp(wq_hbm.reshape(M * H, D), wq_v, sems.at[0]),
            cp(x_hbm, x_v, sems.at[0]),
            cp(wuk_hbm.reshape(DC * H, D), wuk_v, sems.at[0]),
        ]
        wuv_copy = cp(wuv_hbm.reshape(DC * H, D), wuv_v, sems.at[SEM_KV[1]])
        ffn_copies = [
            cp(b1_hbm, b1_v, sems.at[1]),
            cp(b2_hbm, b2_v, sems.at[1]),
            cp(w1_hbm, w1_v, sems.at[1]),
            cp(w2_hbm, w2_v, sems.at[1]),
        ]

        for c in q_copies:
            c.start()
        for j in range(len(KV_SPLITS[0])):
            kv_copy(0, j).start()
        wuv_copy.start()
        for j in range(len(KV_SPLITS[1])):
            kv_copy(1, j).start()
        for c in ffn_copies:
            c.start()
        for i in range(NWO):
            wo_copy(i).start()

        grp_row_d = lax.broadcasted_iota(jnp.int32, (8, D), 0) // B
        grp_row_c = lax.broadcasted_iota(jnp.int32, (8, DC), 0) // B

        for c in q_copies:
            c.wait()
        x = x_v[...].astype(F32)
        mu = jnp.mean(x, axis=-1, keepdims=True)
        xc = x - mu
        var = jnp.mean(xc * xc, axis=-1, keepdims=True)
        xn = xc * lax.rsqrt(var + 1e-5)
        xn8 = jnp.concatenate([xn] * 4, axis=0).astype(BF16)

        def q_body(grp, _):
            for half in range(2):
                q8 = jnp.zeros((8, D), F32)
                for pj in range(2):
                    w = head_pair(wq_v, grp, 2 * half + pj)
                    for hh in range(2):
                        r = jnp.dot(xn8, w[hh], preferred_element_type=F32)
                        q8 = jnp.where(grp_row_d == 2 * pj + hh, r, q8)
                q8 = q8.astype(BF16)
                qa8 = jnp.zeros((8, DC), F32)
                for pj in range(2):
                    w = head_pair(wuk_v, grp, 2 * half + pj)
                    for hh in range(2):
                        r = lax.dot_general(q8, w[hh], NT,
                                            preferred_element_type=F32)
                        qa8 = jnp.where(grp_row_c == 2 * pj + hh, r, qa8)
                rows = pl.ds(pl.multiple_of(16 * grp + 8 * half, 8), 8)
                for ct in range(CT):
                    qa_v[ct, rows, :] = qa8[:, LANES * ct:LANES * (ct + 1)]
            return 0

        lax.fori_loop(0, H // 8, q_body, 0)
        for b in range(B):
            qa = jnp.concatenate(
                [qa_v[ct, pl.ds(b, H, stride=B), :] for ct in range(CT)], axis=1)
            qb_v[b] = (qa * (D ** -0.5 * LOG2E)).astype(BF16)

        for b in range(B):
            def kv_body(t, carry, b=b):
                m, l, acc = carry
                c = kv_v[b, pl.ds(pl.multiple_of(t * TK, TK), TK), :]
                s = lax.dot_general(qb_v[b], c, NT, preferred_element_type=F32)
                m_new = jnp.maximum(m, jnp.max(s, axis=-1, keepdims=True))
                alpha = jnp.exp2(m - m_new)
                p = jnp.exp2(s - m_new)
                l = alpha * l + jnp.sum(p, axis=-1, keepdims=True)
                acc = alpha * acc + jnp.dot(p.astype(BF16), c,
                                            preferred_element_type=F32)
                return m_new, l, acc

            carry = (jnp.full((H, 1), -jnp.inf, F32), jnp.zeros((H, 1), F32),
                     jnp.zeros((H, DC), F32))
            for j in range(len(KV_SPLITS[b])):
                kv_copy(b, j).wait()
                if b == 1 and j == 0:
                    wuv_copy.wait()
                t0 = sum(KV_SPLITS[b][:j]) // TK
                carry = lax.fori_loop(t0, t0 + KV_SPLITS[b][j] // TK,
                                      kv_body, carry)
            _, l, acc = carry
            o = acc / l
            for ct in range(CT):
                olat_v[ct, pl.ds(b, H, stride=B), :] = (
                    o[:, LANES * ct:LANES * (ct + 1)])

        def ctx_body(grp, _):
            for half in range(2):
                rows = pl.ds(pl.multiple_of(16 * grp + 8 * half, 8), 8)
                o8 = jnp.concatenate(
                    [olat_v[ct, rows, :] for ct in range(CT)],
                    axis=1).astype(BF16)
                c8 = jnp.zeros((8, D), F32)
                for pj in range(2):
                    w = head_pair(wuv_v, grp, 2 * half + pj)
                    for hh in range(2):
                        r = jnp.dot(o8, w[hh], preferred_element_type=F32)
                        c8 = jnp.where(grp_row_d == 2 * pj + hh, r, c8)
                ctx_v[rows, :] = c8
            return 0

        lax.fori_loop(0, H // 8, ctx_body, 0)

        for c in ffn_copies:
            c.wait()
        hid = (jnp.dot(xn8, w1_v[...], preferred_element_type=F32)
               + b1_v[...].astype(F32).reshape(1, F))
        hid = jax.nn.gelu(hid, approximate=True).astype(BF16)
        y = (jnp.dot(hid, w2_v[...], preferred_element_type=F32)
             + b2_v[...].astype(F32).reshape(1, M))
        gate = (y * jax.nn.sigmoid(y))[0:B]

        def head_term(c8, hh, h):
            cm = jnp.where(grp_row_d == hh, c8, 0.0).astype(BF16)
            return jnp.dot(cm, wo_v[h], preferred_element_type=F32)

        def wo_body(i, s8):
            c8 = ctx_v[pl.ds(pl.multiple_of(8 * i, 8), 8), :]
            for hh in range(4):
                s8 = s8 + head_term(c8, hh, 4 * i + hh)
            return s8

        s8 = jnp.zeros((8, M), F32)
        for i in range(NWO):
            wo_copy(i).wait()
            lo, hi = WO_SPLITS[i], WO_SPLITS[i + 1]
            if lo % 4 == 0 and hi % 4 == 0:
                s8 = lax.fori_loop(lo // 4, hi // 4, wo_body, s8)
            else:
                for h in range(lo, hi):
                    s8 = s8 + head_term(ctx_v[pl.ds(8 * (h // 4), 8), :],
                                        h % 4, h)
        s = s8[0:2] + s8[2:4] + s8[4:6] + s8[6:8]
        o_ref[...] = (x + s * gate).astype(o_ref.dtype)

    hbm = pl.BlockSpec(memory_space=pl.ANY)
    out = pl.pallas_call(
        kernel,
        out_shape=jax.ShapeDtypeStruct((B, M), A_x.dtype),
        in_specs=[hbm] * 10,
        out_specs=pl.BlockSpec(memory_space=pltpu.VMEM),
        scratch_shapes=[
            pltpu.VMEM((B, M), BF16),
            pltpu.VMEM((B, SK, DC), BF16),
            pltpu.VMEM((M * H, D), BF16),
            pltpu.VMEM((DC * H, D), BF16),
            pltpu.VMEM((DC * H, D), BF16),
            pltpu.VMEM((H, D, M), BF16),
            pltpu.VMEM((M, F), BF16),
            pltpu.VMEM((F,), BF16),
            pltpu.VMEM((F, M), BF16),
            pltpu.VMEM((M,), BF16),
            pltpu.VMEM((CT, B * H, LANES), F32),
            pltpu.VMEM((B, H, DC), BF16),
            pltpu.VMEM((CT, B * H, LANES), F32),
            pltpu.VMEM((B * H, D), F32),
            pltpu.SemaphoreType.DMA((NSEM,)),
        ],
        compiler_params=pltpu.CompilerParams(vmem_limit_bytes=100 * 2**20),
    )(A_x.reshape(B, M), A_c_kv, A_w_q, A_w_uk, A_w_uv, A_w_o,
      B_w1, B_b1, B_w2, B_b2)
    return out.reshape(B, SQ, M)
```
